```python
import os as _os
_os.environ.setdefault("JAX_PLATFORMS", "cpu")
import jax
import jax.numpy as jnp

def _softmax(x, axis=-1):
    return jax.nn.softmax(x, axis=axis)
def _gelu(x):
    return jax.nn.gelu(x, approximate=True)
def _silu(x):
    return jax.nn.silu(x)
def _sigmoid(x):
    return jax.nn.sigmoid(x)
def _layernorm(x, axis=-1, eps=1e-5):
    m = jnp.mean(x, axis=axis, keepdims=True)
    v = jnp.var(x, axis=axis, keepdims=True)
    return (x - m) / jnp.sqrt(v + eps)
def _scatter_add(tgt, idx, src, axis=0):
    return tgt.at[idx].add(src)
def _segment_sum(src, seg, n):
    return jax.ops.segment_sum(src, seg, n)
class _Rng:
    def __init__(self, key):
        self._k = key
    def _next(self):
        self._k, sub = jax.random.split(self._k)
        return sub
    def normal(self, shape):
        return jax.random.normal(self._next(), shape, dtype=jnp.bfloat16)
    def randint(self, lo, hi, shape):
        return jax.random.randint(self._next(), shape, lo, hi, dtype=jnp.int32)
    def uniform(self, shape, lo=0.0, hi=1.0):
        return jax.random.uniform(self._next(), shape, jnp.bfloat16, lo, hi)
    def permutation(self, n):
        return jax.random.permutation(self._next(), n)


kernel_name = 'interleave_layers__sliding_block__dense_activation_gelu__prompt'

def setup_inputs():
    _rng = _Rng(jax.random.key(int.from_bytes(__import__("os").urandom(4), "little")))
    _w = (lambda a: (lambda t: t.astype(jnp.bfloat16) if jnp.issubdtype(t.dtype, jnp.floating) else t)(jnp.asarray(a)))
    def _A_setup():
        B, S, D = 1, 2048, 640
        return {
            "x": _w((lambda *s: _rng.normal(s) * 0.05)(B, S, D)),
            "wqkv": _w((lambda *s: _rng.normal(s) * 0.05)(D, 3 * D)),
            "wo": _w((lambda *s: _rng.normal(s) * 0.05)(D, D)),
        }
    _A_in = _A_setup()

    def _B_setup():
        B, S, D, F = 1, 2048, 640, 1728
        return {
            "x": _w((lambda *s: _rng.normal(s) * 0.05)(B, S, D)),
            "w1": _w((lambda *s: _rng.normal(s) * 0.8)(D, F) * (D ** -0.5)),
            "b1": _w((lambda *s: _rng.normal(s) * 0.8)(F) * 0.01),
            "w2": _w((lambda *s: _rng.normal(s) * 0.8)(F, D) * (F ** -0.5)),
            "b2": _w((lambda *s: _rng.normal(s) * 0.8)(D) * 0.01),
        }
    _B_in = _B_setup()

    return {
        "A_x": _A_in["x"],
        "A_wqkv": _A_in["wqkv"],
        "A_wo": _A_in["wo"],
        "B_x": _B_in["x"],
        "B_w1": _B_in["w1"],
        "B_b1": _B_in["b1"],
        "B_w2": _B_in["w2"],
        "B_b2": _B_in["b2"],
    }

def reference(A_x, A_wqkv, A_wo, B_x, B_w1, B_b1, B_w2, B_b2):
    def _A_ref(x, wqkv, wo):
        B, S, D = x.shape
        H = 32; Dh = D // H; W = 256
        qkv = (lambda x, *d: x.transpose(*d))((x @ wqkv).reshape(B, S, 3, H, Dh), 2, 0, 3, 1, 4)
        q, k, v = qkv[0], qkv[1], qkv[2]
        scores = jnp.einsum("bhqd,bhkd->bhqk", q, k) * (Dh ** -0.5)
        idx = jnp.arange(S)
        mask = (idx[:, None] - idx[None, :] >= 0) & (idx[:, None] - idx[None, :] < W)
        scores = jnp.where(mask[None, None], scores, -1e9)
        p = _softmax(scores, axis=-1)
        o = jnp.einsum("bhqk,bhkd->bhqd", p, v)
        return (lambda x, *d: x.transpose(*d))(o, 0, 2, 1, 3).reshape(B, S, D) @ wo

    def _B_ref(x, w1, b1, w2, b2):
        h = jnp.einsum("bsd,df->bsf", x, w1) + b1
        h = _gelu(h)
        return jnp.einsum("bsf,fd->bsd", h, w2) + b2

    x = A_x
    x = x + _A_ref(_layernorm(x, axis=-1), A_wqkv, A_wo)
    x = x + _B_ref(_layernorm(x, axis=-1), B_w1, B_b1, B_w2, B_b2)
    x = x + _A_ref(_layernorm(x, axis=-1), A_wqkv, A_wo)
    x = x + _B_ref(_layernorm(x, axis=-1), B_w1, B_b1, B_w2, B_b2)
    return x
```

```python
import functools
import jax
import jax.numpy as jnp
from jax import lax
import jax.experimental.pallas as pl
import jax.experimental.pallas.tpu as pltpu

S, D, H, DH, W, F = 2048, 640, 32, 20, 256, 1728
QB = 128
NEG = -1e30
BF = jnp.bfloat16
F32 = jnp.float32
NT = (((1,), (1,)), ((), ()))


def _ln(x):
    m = jnp.mean(x, axis=-1, keepdims=True)
    xc = x - m
    v = jnp.mean(xc * xc, axis=-1, keepdims=True)
    return xc * lax.rsqrt(v + 1e-5)


def _gelu(x):
    c = 0.7978845608028654
    return 0.5 * x * (1.0 + jnp.tanh(c * (x + 0.044715 * (x * x * x))))


def make_kernel(T, attn, dense, G):
    nq = T // QB

    def kernel(x_ref, wqkv_h, wo_h, w1t_h, b1_ref, w2_h, b2_ref, o_ref,
               kbuf, vtbuf, otbuf, sbuf, mbuf, wqkv_ref, wvt_ref, wo_ref, w1t_ref, w2_ref, sems):
        i = pl.program_id(0)

        cps = [pltpu.make_async_copy(a, b, sems.at[n]) for n, (a, b) in enumerate(
            [(wqkv_h, wqkv_ref), (wo_h, wo_ref), (w1t_h, w1t_ref), (w2_h, w2_ref)])]

        @pl.when(i == 0)
        def _():
            for c in cps:
                c.start()
            kbuf[0:W, :] = jnp.zeros((W, D), BF)
            kbuf[S + W:S + 2 * W, :] = jnp.zeros((W, D), BF)
            vtbuf[:, :, :, 0:W] = jnp.zeros((2, H, 32, W), BF)
            cps[0].wait()
            wvt_ref[...] = wqkv_ref[:, 2 * D:3 * D].astype(F32).T.astype(BF)
            cps[1].wait()
            cps[2].wait()
            cps[3].wait()

        r_io = lax.broadcasted_iota(jnp.int32, (QB, QB), 0)
        c_io = lax.broadcasted_iota(jnp.int32, (QB, QB), 1)
        tri = r_io <= c_io

        def attn_qb(l, qt, t0, qs, first):
            t0 = pl.multiple_of(t0, QB)
            for g in range(H // G):
                for hh in range(G):
                    h = g * G + hh
                    lo, hi = h * DH, (h + 1) * DH
                    s0 = lo // 128
                    s1 = (hi - 1) // 128
                    qs_ = qt[qs * QB:(qs + 1) * QB, s0 * 128:(s1 + 1) * 128]
                    lio = lax.broadcasted_iota(jnp.int32, qs_.shape, 1) + s0 * 128
                    qw = jnp.where((lio >= lo) & (lio < hi), qs_, 0.0).astype(BF)
                    kw = kbuf[pl.ds(pl.multiple_of(l * (S + W) + t0, QB), 3 * QB), s0 * 128:(s1 + 1) * 128]
                    st = lax.dot_general(kw, qw, NT, preferred_element_type=F32)
                    far, mid, dia = st[0:QB], st[QB:2 * QB], st[2 * QB:3 * QB]
                    if first and qs == 0:
                        far = jnp.full_like(far, NEG)
                        mid = jnp.full_like(mid, NEG)
                    elif first and qs == 1:
                        far = jnp.full_like(far, NEG)
                    mg = jnp.where(tri, dia, far)
                    m = jnp.max(jnp.maximum(mg, mid), axis=0, keepdims=True)
                    sbuf[hh, 0:QB, :] = mg
                    sbuf[hh, QB:2 * QB, :] = mid
                    mbuf[hh] = jnp.broadcast_to(m, (8, QB))
                for hh in range(G):
                    h = g * G + hh
                    m = mbuf[hh][0:1]
                    pm = jnp.exp2(sbuf[hh, 0:QB, :] - m)
                    pmid = jnp.exp2(sbuf[hh, QB:2 * QB, :] - m)
                    pd = jnp.where(tri, pm, 0.0)
                    pf = jnp.where(tri, 0.0, pm)
                    pt = jnp.concatenate([pf, pmid, pd], axis=0).astype(BF)
                    vt = vtbuf[l, h, :, pl.ds(t0, 3 * QB)]
                    ot = jnp.dot(vt, pt, preferred_element_type=F32)
                    o = ot[0:24] * (1.0 / ot[24:25])
                    otbuf[h, :, qs * QB:(qs + 1) * QB] = o

        def layer(l, x, first):
            t0 = pl.multiple_of(i * T, T)
            xn = _ln(x).astype(BF)
            k = jnp.dot(xn, wqkv_ref[:, D:2 * D], preferred_element_type=F32)
            kbuf[pl.ds(pl.multiple_of(l * (S + W) + t0 + W, QB), T), :] = k.astype(BF)
            qt = jnp.dot(xn, wqkv_ref[:, 0:D], preferred_element_type=F32)
            qt = qt * (DH ** -0.5 * 1.4426950408889634)
            vt = lax.dot_general(wvt_ref[...], xn, NT, preferred_element_type=F32)
            rio = lax.broadcasted_iota(jnp.int32, (32, T), 0)
            for h in range(H):
                lo = h * DH
                if lo + 32 <= D:
                    pc = vt[lo:lo + 32]
                    pc = jnp.where(rio < DH, pc, jnp.where(rio >= 24, 1.0, 0.0))
                else:
                    pc = jnp.concatenate([vt[lo:lo + DH], jnp.zeros((4, T), F32), jnp.ones((8, T), F32)], axis=0)
                vtbuf[l, h, :, pl.ds(t0 + W, T)] = pc.astype(BF)
            if attn:
                for qs in range(nq):
                    attn_qb(l, qt, t0 + qs * QB, qs, first)
                ot = jnp.concatenate([otbuf[h, 0:DH, :] for h in range(H)], axis=0)
                o = ot.T.astype(BF)
            else:
                o = qt.astype(BF)
            x = x + jnp.dot(o, wo_ref[...], preferred_element_type=F32)
            if dense:
                xn = _ln(x).astype(BF)
                hh = lax.dot_general(xn, w1t_ref[...], NT, preferred_element_type=F32) + b1_ref[...]
                hh = _gelu(hh).astype(BF)
                x = x + jnp.dot(hh, w2_ref[...], preferred_element_type=F32) + b2_ref[...]
            return x

        def run(first):
            x = x_ref[...].astype(F32)
            x = lax.fori_loop(0, 2, lambda l, x: layer(l, x, first), x)
            o_ref[...] = x.astype(o_ref.dtype)

        pl.when(i == 0)(lambda: run(True))
        pl.when(i > 0)(lambda: run(False))

    return kernel


@jax.jit
def pallas_interleave_layers__sliding_block__dense_activation_gelu__prompt_kernel(A_x, A_wqkv, A_wo, B_x, B_w1, B_b1, B_w2, B_b2):
    T = 256
    attn = True
    dense = True
    G = 32
    x = A_x.reshape(S, D)
    b1 = B_b1.reshape(1, F)
    b2 = B_b2.reshape(1, D)
    args = (x, A_wqkv, A_wo, B_w1.T, b1, B_w2, b2)
    full = lambda a: pl.BlockSpec(a.shape, lambda i: (0,) * a.ndim)
    hbm = pl.BlockSpec(memory_space=pl.ANY)
    out = pl.pallas_call(
        make_kernel(T, attn, dense, G),
        grid=(S // T,),
        in_specs=[pl.BlockSpec((T, D), lambda i: (i, 0))] + [hbm, hbm, hbm, full(b1), hbm, full(b2)],
        out_specs=pl.BlockSpec((T, D), lambda i: (i, 0)),
        out_shape=jax.ShapeDtypeStruct((S, D), A_x.dtype),
        scratch_shapes=[pltpu.VMEM((2 * (S + W), D), BF), pltpu.VMEM((2, H, 32, S + W), BF),
                        pltpu.VMEM((H, 24, T), F32), pltpu.VMEM((G, 2 * QB, QB), F32), pltpu.VMEM((G, 8, QB), F32),
                        pltpu.VMEM((D, 3 * D), BF), pltpu.VMEM((D, D), BF), pltpu.VMEM((D, D), BF),
                        pltpu.VMEM((F, D), BF), pltpu.VMEM((F, D), BF), pltpu.SemaphoreType.DMA((4,))],
        compiler_params=pltpu.CompilerParams(dimension_semantics=("arbitrary",),
                                             vmem_limit_bytes=100 * 1024 * 1024),
    )(*args)
    return out.reshape(1, S, D)
```

```python
import functools
import jax
import jax.numpy as jnp
from jax import lax
import jax.experimental.pallas as pl
import jax.experimental.pallas.tpu as pltpu

S, D, H, DH, W, F = 2048, 640, 32, 20, 256, 1728
QB = 128
NEG = -1e30
BF = jnp.bfloat16
F32 = jnp.float32
NP = 16
U32 = jnp.uint32


def _pk(x):
    return pltpu.bitcast(x.astype(BF), U32)


def _sh(x):
    x = _pk(x)
    return jnp.concatenate([x, x[:, 64:576]], axis=1)

NT = (((1,), (1,)), ((), ()))


def _ln(x):
    m = jnp.mean(x, axis=-1, keepdims=True)
    xc = x - m
    v = jnp.mean(xc * xc, axis=-1, keepdims=True)
    return xc * lax.rsqrt(v + 1e-5)


def _gelu(x):
    c = 0.7978845608028654
    return 0.5 * x * (1.0 + jnp.tanh(c * (x + 0.044715 * (x * x * x))))


def when0(l, f):
    if isinstance(l, int):
        if l == 0:
            f()
    else:
        pl.when(l == 0)(f)


def make_kernel(T, attn, dense, G, FC, UNR, NH, ROLL, PRE, WALL, L2, SEQ, NC, DB, BAR):
    nq = T // QB

    def kernel(x_ref, xnext_ref, wqkv_h, wo_h, w1t_h, b1_ref, w2_h, b2_ref, o_ref,
               kbuf, vtbuf, otbuf, sbuf, mbuf, wqkv_ref, wvt_ref, wo_ref, w1t_ref, w2_ref, w1n_ref, qbuf, xnbuf, sems):
        i = pl.program_id(0)

        class Multi:
            def __init__(self, a, b, n):
                r = a.shape[0] // NC
                self.c = [pltpu.make_async_copy(a.at[pl.ds(k * r, r)], b.at[pl.ds(k * r, r)], sems.at[n * NC + k]) for k in range(NC)]

            def start(self):
                for c in self.c:
                    c.start()

            def wait(self):
                for c in self.c:
                    c.wait()

        cps = [Multi(a, b, n) for n, (a, b) in enumerate(
            [(wqkv_h, wqkv_ref), (wo_h, wo_ref), (w1t_h, w1t_ref), (w2_h, w2_ref)])]

        @pl.when(i == 0)
        def _():
            cps[0].start()
            if not SEQ:
                for c in cps[1:]:
                    c.start()
            kbuf[0:W // 2, :] = jnp.zeros((W // 2, D + 512), U32)
            kbuf[(S + W) // 2:(S + 2 * W) // 2, :] = jnp.zeros((W // 2, D + 512), U32)
            vtbuf[:, :, :, 0:W] = jnp.zeros((2, NP, 24, W), U32)
            xnbuf[...] = _ln(x_ref[...].astype(F32)).astype(BF)
            cps[0].wait()
            if SEQ:
                for c in cps[1:]:
                    c.start()
            if WALL:
                cps[1].wait()
                cps[2].wait()
                cps[3].wait()
            wvt_ref[...] = wqkv_ref[:, 2 * D:3 * D].astype(F32).T.astype(BF)

        r_io = lax.broadcasted_iota(jnp.int32, (64, 128), 0)
        c_io = lax.broadcasted_iota(jnp.int32, (64, 128), 1)
        tri = r_io <= jnp.where(c_io >= 64, c_io - 64, c_io)

        def attn_qb(l, t0, jj, first, ph=3):
            base = pl.multiple_of(l * (S + W) // 2 + i * (T // 2) + jj * 64, 64)
            for g in range(NP // G):
                for pp in range(G if ph & 1 else 0):
                    p = g * G + pp
                    lo = 40 * p
                    if lo // 128 == (lo + 39) // 128:
                        sl = lo // 128
                        fb, kc = sl * 128, sl * 128
                        qc = sl * 128
                    else:
                        sl = (lo - 64) // 128
                        fb, kc = 64 + sl * 128, D + sl * 128
                        qc = sl * 128
                    for b in range(2):
                        j = 2 * jj + b
                        q64 = pltpu.bitcast(qbuf[j * 32:j * 32 + 32, kc:kc + 128], BF)
                        lio = lax.broadcasted_iota(jnp.int32, q64.shape, 1) + fb
                        q0 = jnp.where((lio >= lo) & (lio < lo + 20), q64, jnp.zeros_like(q64))
                        q1 = jnp.where((lio >= lo + 20) & (lio < lo + 40), q64, jnp.zeros_like(q64))
                        qw = jnp.concatenate([q0, q1] if b == 0 else [q1, q0], axis=0)
                        kw = pltpu.bitcast(kbuf[pl.ds(pl.multiple_of(base + 32 * b, 32), 160), kc:kc + 128], BF)
                        st = lax.dot_general(kw, qw, NT, preferred_element_type=F32)
                        far, mid, dia = st[0:64], st[64:256], st[256:320]
                        thr = W - (t0 + 64 * b)
                        far = jnp.where(r_io >= thr, far, NEG)
                        mid = jnp.concatenate([jnp.where(r_io >= thr - 64 * (n + 1), mid[64 * n:64 * n + 64], NEG) for n in range(3)], axis=0)
                        mg = jnp.where(tri, dia, far)
                        m = jnp.maximum(jnp.maximum(mg, mid[0:64]), jnp.maximum(mid[64:128], mid[128:192]))
                        m = jnp.max(m, axis=0, keepdims=True)
                        u = 2 * pp + b + (2 * G * jj if DB else 0)
                        sbuf[u, 0:64, :] = mg
                        sbuf[u, 64:256, :] = mid
                        mbuf[u] = jnp.broadcast_to(m, (8, 128))
                for pp in range(G if ph & 2 else 0):
                    p = g * G + pp
                    res = []
                    for b in range(2):
                        u = 2 * pp + b + (2 * G * jj if DB else 0)
                        m = mbuf[u][0:1]
                        pm = jnp.exp2(sbuf[u, 0:64, :] - m)
                        pmid = jnp.exp2(sbuf[u, 64:256, :] - m)
                        pd = jnp.where(tri, pm, 0.0)
                        pf = jnp.where(tri, 0.0, pm)
                        pt = jnp.concatenate([pf, pmid, pd], axis=0).astype(BF)
                        vt = pltpu.bitcast(vtbuf[l, p, :, pl.ds(pl.multiple_of(t0, QB), 384)], BF)
                        vt = vt[:, 0:320] if b == 0 else vt[:, 64:384]
                        res.append(jnp.dot(vt, pt, preferred_element_type=F32))
                    A, B = res
                    rr = lax.broadcasted_iota(jnp.int32, (48, 128), 0)
                    cc = lax.broadcasted_iota(jnp.int32, (48, 128), 1)
                    e0 = jnp.where(cc < 64, A, B)
                    e1 = pltpu.roll(jnp.where(cc < 64, B, A), 64, 1)
                    h0 = (rr < 20) | ((rr >= 40) & (rr < 44))
                    e = jnp.where(h0, e0, e1)
                    inv = 1.0 / e[40:48]
                    r40 = lax.broadcasted_iota(jnp.int32, (40, 128), 0)
                    o = e[0:40] * jnp.where(r40 < 20, inv[0:1], inv[4:5])
                    otbuf[40 * p:40 * p + 40, pl.ds(pl.multiple_of(jj * QB, QB), QB)] = o

        def layer(l, x, first):
            t0 = pl.multiple_of(i * T, T)
            xn = xnbuf[...] if l == 0 else (jnp.concatenate([_ln(x[n * 128:n * 128 + 128]).astype(BF) for n in range(2)], axis=0) if L2 else _ln(x).astype(BF))
            k = jnp.dot(xn, wqkv_ref[:, D:2 * D], preferred_element_type=F32)
            kbuf[pl.ds(pl.multiple_of((l * (S + W) + W) // 2 + i * (T // 2), 64), T // 2), :] = _sh(k)
            qt = jnp.dot(xn, wqkv_ref[:, 0:D], preferred_element_type=F32)
            qt = qt * (DH ** -0.5 * 1.4426950408889634)
            vt = lax.dot_general(wvt_ref[...], xn, NT, preferred_element_type=F32)
            for p in range(NP):
                pc = jnp.concatenate([vt[40 * p:40 * p + 40], jnp.ones((8, T), F32)], axis=0)
                vtbuf[l, p, :, pl.ds(t0 + W, T)] = _pk(pc)
            if attn:
                qbuf[...] = _sh(qt)
                if l == 1 and PRE == 3:
                    xnbuf[...] = _ln(xnext_ref[...].astype(F32)).astype(BF)
                if not ROLL:
                    if DB == 2:
                        for qs, ph in ((0, 1), (1, 1), (0, 2), (1, 2)):
                            attn_qb(l, t0 + qs * QB, qs, first, ph)
                            if l == 0 and BAR == 1 and (qs, ph) == (1, 1):
                                @pl.when(i == 0)
                                def _():
                                    cps[1].wait()
                                    cps[2].wait()
                                    cps[3].wait()
                    else:
                        for qs in range(nq):
                            attn_qb(l, t0 + qs * QB, qs, first)
                else:
                    lax.fori_loop(0, nq, lambda qs, c: (attn_qb(l, t0 + qs * QB, qs, False), c)[1], 0)
                ot = otbuf[...]
                o = ot.T.astype(BF)
            else:
                o = qt.astype(BF)
            if l == 0 and BAR == 0:
                @pl.when(i == 0)
                def _():
                    cps[1].wait()
                    cps[2].wait()
                    cps[3].wait()
            HS = T // NH
            xs = [x[n * HS:(n + 1) * HS] + jnp.dot(o[n * HS:(n + 1) * HS], wo_ref[...], preferred_element_type=F32) for n in range(NH)]
            if dense:
                xns = [_ln(xx).astype(BF) for xx in xs]
                outs = []
                for n in range(NH):
                    acc = xs[n] + b2_ref[...].astype(F32).reshape(1, D)
                    if l == 1 and n == NH - 1 and PRE == 1:
                        xnbuf[...] = _ln(xnext_ref[...].astype(F32)).astype(BF)
                    if l == 1 and PRE == 2:
                        xnbuf[n * HS:(n + 1) * HS] = _ln(xnext_ref[n * HS:(n + 1) * HS].astype(F32)).astype(BF)
                    for f0 in range(0, F, FC):
                        f1 = min(F, f0 + FC)
                        hh = lax.dot_general(xns[n], w1t_ref[f0:f1, :], NT, preferred_element_type=F32) + b1_ref[...].astype(F32).reshape(1, F)[:, f0:f1]
                        hh = _gelu(hh).astype(BF)
                        acc = acc + jnp.dot(hh, w2_ref[f0:f1, :], preferred_element_type=F32)
                    outs.append(acc)
                xs = outs
            x = jnp.concatenate(xs, axis=0) if NH > 1 else xs[0]
            return x

        def run(first):
            x = x_ref[...].astype(F32)
            if UNR:
                x = layer(1, layer(0, x, first), first)
            else:
                x = lax.fori_loop(0, 2, lambda l, x: layer(l, x, first), x)
            o_ref[...] = x.astype(o_ref.dtype)

        run(False)

    return kernel


@jax.jit
def pallas_interleave_layers__sliding_block__dense_activation_gelu__prompt_kernel(A_x, A_wqkv, A_wo, B_x, B_w1, B_b1, B_w2, B_b2):
    T = 256
    attn = True
    dense = True
    G = 16
    FC = 1728
    UNR = True
    NH = 4
    ROLL = False
    PRE = 2
    WALL = False
    L2 = False
    SEQ = True
    NC = 1
    GR = 8
    FL = ()
    DB = 2
    BAR = 1
    x = A_x.reshape(S, D)
    b1 = B_b1
    b2 = B_b2
    args = (x, x, A_wqkv, A_wo, B_w1.T, b1, B_w2, b2)
    full = lambda a: pl.BlockSpec(a.shape, lambda i: (0,) * a.ndim)
    hbm = pl.BlockSpec(memory_space=pl.ANY)
    out = pl.pallas_call(
        make_kernel(T, attn, dense, G, FC, UNR, NH, ROLL, PRE, WALL, L2, SEQ, NC, DB, BAR),
        grid=(GR,),
        in_specs=[pl.BlockSpec((T, D), lambda i: (i, 0)), pl.BlockSpec((T, D), lambda i: (jnp.minimum(i + 1, S // T - 1), 0))] + [hbm, hbm, hbm, full(b1), hbm, full(b2)],
        out_specs=pl.BlockSpec((T, D), lambda i: (i, 0)),
        out_shape=jax.ShapeDtypeStruct((S, D), A_x.dtype),
        scratch_shapes=[pltpu.VMEM((S + W, D + 512), U32), pltpu.VMEM((2, NP, 24, S + W), U32),
                        pltpu.VMEM((D, T), F32), pltpu.VMEM((4 * G, 2 * QB, QB), F32), pltpu.VMEM((4 * G, 8, QB), F32),
                        pltpu.VMEM((D, 3 * D), BF), pltpu.VMEM((D, D), BF), pltpu.VMEM((D, D), BF),
                        pltpu.VMEM((F, D), BF), pltpu.VMEM((F, D), BF), pltpu.VMEM((8, 128), BF), pltpu.VMEM((T // 2, D + 512), U32), pltpu.VMEM((T, D), BF), pltpu.SemaphoreType.DMA((4 * NC,))],
        compiler_params=pltpu.CompilerParams(flags=dict(FL) if FL else None, dimension_semantics=("arbitrary",),
                                             vmem_limit_bytes=100 * 1024 * 1024),
    )(*args)
    return out.reshape(1, S, D)
```
